```python
import os as _os
_os.environ.setdefault("JAX_PLATFORMS", "cpu")
import jax
import jax.numpy as jnp

def _softmax(x, axis=-1):
    return jax.nn.softmax(x, axis=axis)
def _gelu(x):
    return jax.nn.gelu(x, approximate=True)
def _silu(x):
    return jax.nn.silu(x)
def _sigmoid(x):
    return jax.nn.sigmoid(x)
def _layernorm(x, axis=-1, eps=1e-5):
    m = jnp.mean(x, axis=axis, keepdims=True)
    v = jnp.var(x, axis=axis, keepdims=True)
    return (x - m) / jnp.sqrt(v + eps)
def _scatter_add(tgt, idx, src, axis=0):
    return tgt.at[idx].add(src)
def _segment_sum(src, seg, n):
    return jax.ops.segment_sum(src, seg, n)
class _Rng:
    def __init__(self, key):
        self._k = key
    def _next(self):
        self._k, sub = jax.random.split(self._k)
        return sub
    def normal(self, shape):
        return jax.random.normal(self._next(), shape, dtype=jnp.bfloat16)
    def randint(self, lo, hi, shape):
        return jax.random.randint(self._next(), shape, lo, hi, dtype=jnp.int32)
    def uniform(self, shape, lo=0.0, hi=1.0):
        return jax.random.uniform(self._next(), shape, jnp.bfloat16, lo, hi)
    def permutation(self, n):
        return jax.random.permutation(self._next(), n)


kernel_name = 'standalone__gqa_block_cached__near_ridge'

def setup_inputs():
    _rng = _Rng(jax.random.key(int.from_bytes(__import__("os").urandom(4), "little")))
    _w = (lambda a: (lambda t: t.astype(jnp.bfloat16) if jnp.issubdtype(t.dtype, jnp.floating) else t)(jnp.asarray(a)))
    B, Sq, D = 8, 64, 512
    Hq, Hkv, Sk, Dh = 32, 8, 64, 128
    assert Hq % Hkv == 0, (Hq, Hkv)
    return {
        "x": _w((lambda *s: _rng.normal(s) * 0.8)(B, Sq, D)),
        "k_cache": _w((lambda *s: _rng.normal(s) * 0.8)(B, Hkv, Sk, Dh)),
        "v_cache": _w((lambda *s: _rng.normal(s) * 0.05)(B, Hkv, Sk, Dh)),
        "wq": _w((lambda *s: _rng.normal(s) * 0.8)(D, Hq * Dh) * (D ** -0.5)),
        "wo": _w((lambda *s: _rng.normal(s) * 0.05)(Hq * Dh, D) * ((Hq * Dh) ** -0.5)),
    }

def reference(x, k_cache, v_cache, wq, wo):
    B, Sq, D = x.shape
    Hq, Dh = 32, 128
    Hkv = k_cache.shape[1]
    rep = Hq // Hkv
    q = (lambda x, *d: x.transpose(*d))((x @ wq).reshape(B, Sq, Hq, Dh), 0, 2, 1, 3)
    k = jnp.repeat(k_cache, rep, axis=1)
    v = jnp.repeat(v_cache, rep, axis=1)
    scores = jnp.einsum("bhqd,bhkd->bhqk", q, k) * (Dh ** -0.5)
    p = _softmax(scores, axis=-1)
    o = jnp.einsum("bhqk,bhkd->bhqd", p, v)
    return (lambda x, *d: x.transpose(*d))(o, 0, 2, 1, 3).reshape(B, Sq, Hq * Dh) @ wo
```

```python
import functools
import jax
import jax.numpy as jnp
import numpy as np
import jax.experimental.pallas as pl
import jax.experimental.pallas.tpu as pltpu

B, SQ, D = 8, 64, 512
HQ, HKV, SK, DH = 32, 8, 64, 128
REP = HQ // HKV
GW = REP * DH
M = B * SQ
LOG2E = 1.4426950408889634
C = np.float32(DH ** -0.5 * LOG2E)
bf16 = jnp.bfloat16
f32 = jnp.float32


def make_kernel(mode, wait_slots, start_plan, sched):
    def _kernel(x_hbm, k_hbm, v_hbm, wq_hbm, wo_hbm, o_hbm,
                x_v, wq_v, wo_v, k_v, v_v, acc, out_v, q_s, p_s, o_s, sx, sq, so, sk, sv, sout):
        cx = pltpu.make_async_copy(x_hbm, x_v, sx.at[0])
        cq = [pltpu.make_async_copy(wq_hbm.at[:, pl.ds(g * GW, GW)], wq_v.at[g], sq.at[g]) for g in range(HKV)]
        co = [pltpu.make_async_copy(wo_hbm.at[pl.ds(g * GW, GW), :], wo_v.at[g], so.at[g]) for g in range(HKV)]
        ck = [pltpu.make_async_copy(k_hbm.at[:, g], k_v.at[g], sk.at[g]) for g in range(HKV)]
        cv = [pltpu.make_async_copy(v_hbm.at[:, g], v_v.at[g], sv.at[g]) for g in range(HKV)]

        def needs(t):
            r = []
            if t == -1:
                r += [cx, cq[0]]
            if 0 <= t < HKV:
                r += [ck[t]]
            if 0 <= t and t + 1 < HKV:
                r += [cq[t + 1]]
            if 0 <= t < HKV:
                r += [cv[t]]
            if 1 <= t <= HKV:
                r += [co[t - 1]]
            return r

        def qproj(g, j0=0, j1=REP):
            if g >= HKV:
                return
            n0, n1 = j0 * DH, j1 * DH
            q = jnp.dot(x_v[...], wq_v[g, :, n0:n1], preferred_element_type=f32)
            q_s[g % 2, :, n0:n1] = q.astype(bf16)

        def qk(g, b):
            if not 0 <= g < HKV:
                return
            q = q_s[g % 2, pl.ds(b * SQ, SQ), :]
            qs = jnp.concatenate([q[:, j * DH:(j + 1) * DH] for j in range(REP)], axis=0)
            if mode == 'rows':
                s = jax.lax.dot_general(qs, k_v[g, b], (((1,), (1,)), ((), ())), preferred_element_type=f32)
                m = jnp.max(s, axis=-1, keepdims=True)
                e = jnp.exp2((s - m) * C)
                l = jnp.sum(e, axis=-1, keepdims=True)
                p_s[b] = (e * pl.reciprocal(l, approx=False, full_range=False)).astype(bf16)
            else:
                st = jax.lax.dot_general(k_v[g, b], qs, (((1,), (1,)), ((), ())), preferred_element_type=f32)
                m = jnp.max(st, axis=0, keepdims=True)
                e = jnp.exp2((st - m) * C)
                l = jnp.sum(e, axis=0, keepdims=True)
                pt = (e * pl.reciprocal(l, approx=False, full_range=False))
                p_s[b] = pt.T.astype(bf16)

        def pv(g, b):
            if not 0 <= g < HKV:
                return
            o = jnp.dot(p_s[b], v_v[g, b], preferred_element_type=f32).astype(bf16)
            for j in range(REP):
                o_s[g % 2, pl.ds(b * SQ, SQ), pl.ds(j * DH, DH)] = o[j * SQ:(j + 1) * SQ, :]

        def outproj(g, j0=0, j1=4):
            if not 0 <= g < HKV:
                return
            n0, n1 = j0 * 128, j1 * 128
            c = jnp.dot(o_s[g % 2], wo_v[g, :, n0:n1], preferred_element_type=f32)
            if g == 0:
                acc[:, n0:n1] = c
            elif g < HKV - 1:
                acc[:, n0:n1] += c
            else:
                out_v[:, n0:n1] = (acc[:, n0:n1] + c).astype(bf16)

        ws = list(wait_slots) + [HKV + 1]
        for c in needs(-1):
            c.start()
        for tt in start_plan.get('pre', []):
            for c in needs(tt):
                c.start()
        for t in range(-1, HKV + 1):
            if t in wait_slots:
                nxt = ws[ws.index(t) + 1]
                for tt in range(t, nxt):
                    for c in needs(tt):
                        c.wait()
            for tt in start_plan.get(t, []):
                for c in needs(tt):
                    c.start()
            for item in sched(t):
                kind = item[0]
                if kind == 'qk':
                    for b in item[1]:
                        qk(t, b)
                elif kind == 'pv':
                    for b in item[1]:
                        pv(t, b)
                elif kind == 'q':
                    qproj(t + 1, item[1], item[2])
                elif kind == 'o':
                    outproj(t - 1, item[1], item[2])
        cout = pltpu.make_async_copy(out_v, o_hbm, sout.at[0])
        cout.start()
        cout.wait()
    return _kernel


def build(mode, wait_slots, start_plan, sched):
    @jax.jit
    def kernel(x, k_cache, v_cache, wq, wo):
        x2 = x.reshape(M, D)
        anyspec = pl.BlockSpec(memory_space=pl.ANY)
        out = pl.pallas_call(
            make_kernel(mode, wait_slots, start_plan, sched),
            in_specs=[anyspec] * 5,
            out_specs=anyspec,
            out_shape=jax.ShapeDtypeStruct((M, D), bf16),
            scratch_shapes=[
                pltpu.VMEM((M, D), bf16),
                pltpu.VMEM((HKV, D, GW), bf16),
                pltpu.VMEM((HKV, GW, D), bf16),
                pltpu.VMEM((HKV, B, SK, DH), bf16),
                pltpu.VMEM((HKV, B, SK, DH), bf16),
                pltpu.VMEM((M, D), f32),
                pltpu.VMEM((M, D), bf16),
                pltpu.VMEM((2, M, GW), bf16),
                pltpu.VMEM((B, REP * SQ, SK), bf16),
                pltpu.VMEM((2, M, GW), bf16),
                pltpu.SemaphoreType.DMA((1,)),
                pltpu.SemaphoreType.DMA((HKV,)),
                pltpu.SemaphoreType.DMA((HKV,)),
                pltpu.SemaphoreType.DMA((HKV,)),
                pltpu.SemaphoreType.DMA((HKV,)),
                pltpu.SemaphoreType.DMA((1,)),
            ],
            compiler_params=pltpu.CompilerParams(vmem_limit_bytes=64 * 1024 * 1024),
        )(x2, k_cache, v_cache, wq, wo)
        return out.reshape(B, SQ, D)
    return kernel


def sched_a(t):
    r = []
    for i in range(4):
        r += [('qk', (2 * i, 2 * i + 1)), ('q', i, i + 1)]
    if t == HKV - 1:
        r += [('o', 0, 3), ('pv', range(8)), ('o', 3, 4)]
    else:
        r += [('pv', range(8)), ('o', 0, 4)]
    return r


def sched_b(t):
    if t == HKV - 1:
        r = []
        for i in range(4):
            r += [('qk', (2 * i, 2 * i + 1))]
            if i < 3:
                r += [('o', i, i + 1)]
        r += [('pv', range(4)), ('o', 3, 4), ('pv', range(4, 8))]
        return r
    r = []
    for i in range(4):
        r += [('qk', (2 * i, 2 * i + 1)), ('q', i, i + 1)]
    r += [('pv', range(4)), ('o', 0, 2), ('pv', range(4, 8)), ('o', 2, 4)]
    return r


_SER = dict(wait_slots=list(range(-1, 9)), start_plan={t: [t + 1] for t in range(-1, 8)})
pallas_standalone__gqa_block_cached__near_ridge_kernel = build('T', sched=sched_b, **_SER)
```

```python
import jax
import jax.numpy as jnp
import numpy as np
import jax.experimental.pallas as pl
import jax.experimental.pallas.tpu as pltpu

B, SQ, D = 8, 64, 512
HQ, HKV, SK, DH = 32, 8, 64, 128
REP = HQ // HKV
GW = REP * DH
M = B * SQ
C = np.float32(DH ** -0.5 * 1.4426950408889634)
bf16 = jnp.bfloat16
f32 = jnp.float32

RX, RWQ, RWO, RK, RV, RPAD, NR = 0, 8, 72, 136, 152, 168, 169


def _x(c):
    return ("x", c)


def _wq(g, r0=0, r1=8, j0=0, j1=4):
    return ("wq", g, r0, r1, j0, j1)


def _needs(t):
    r = []
    if 0 <= t < HKV:
        r.append(("k", t))
    if 0 <= t and t + 1 < HKV:
        r.append(_wq(t + 1))
    if 0 <= t < HKV:
        r.append(("v", t))
    if 1 <= t <= HKV:
        r.append(("wo", t - 1))
    return r


def _slot_steps(order, t):
    steps = []
    for tok in order.split():
        c, arg = tok[0], tok[1:]
        if c == "k" and 0 <= t < HKV:
            steps += [("qk", t, 2 * int(arg)), ("qk", t, 2 * int(arg) + 1)]
        elif c == "q" and 0 <= t and t + 1 < HKV:
            steps.append(("q", t + 1, int(arg)))
        elif c == "p" and 0 <= t < HKV:
            steps += [("pv", t, int(ch)) for ch in arg]
        elif c == "o" and 1 <= t <= HKV:
            steps.append(("o", t - 1, int(arg)))
        elif c == "|":
            steps.append(("fence",))
    return steps


def _schedule():
    sem = {}

    def start(*names):
        return [("start", n, sem.setdefault(n, len(sem))) for n in names]

    def wait(*names):
        return [("wait", n, sem[n]) for n in names]

    def piece(c):
        return (_x(c), _wq(0, 2 * c, 2 * c + 2))

    row = 320
    p = start(*piece(0)) + start(*piece(1))
    p += wait(*piece(0)) + start(*piece(2)) + [("q0", 0), ("pin", ("qacc", 0), row)]
    p += wait(*piece(1)) + start(*piece(3)) + [("q0", 1), ("pin", ("qacc", 1), row)]
    p += wait(*piece(2)) + start(("k", 0), _wq(1, 0, 8, 0, 1)) + [("q0", 2), ("pin", ("qacc", 2), row)]
    p += wait(*piece(3)) + start(_wq(1, 0, 8, 1, 2), _wq(1, 0, 8, 2, 4)) + [("q0", 3)]

    orders = {t: "k0 q0 k1 q1 k2 q2 k3 q3 p0123 o0 o1 p4567 o2 | o3" for t in range(HKV + 1)}
    orders[0] = "| k0 q0 | k1 q1 | k2 q2 | k3 q3 p0123 p4567 |"
    orders[1] = "k0 q0 k1 q1 k2 q2 k3 q3 | p0123 o0 o1 p4567 o2 | o3"
    orders[HKV - 1] = "k0 o0 k1 o1 k2 o2 k3 p0123 | o3 p4567"
    fences = {t: [(None, _needs(t + 1), _needs(t + 2))] for t in range(2, HKV)}
    fences[0] = [
        ((("qacc", 3), row), (("k", 0), _wq(1, 0, 8, 0, 1)), (("v", 0), ("k", 1))),
        ((("q", 1, 0), row), (_wq(1, 0, 8, 1, 2),), (_wq(2),)),
        ((("q", 1, 1), row), (_wq(1, 0, 8, 2, 4),), ()),
        ((("q", 1, 2), row), (("v", 0),), (("v", 1), ("wo", 0))),
        (None, (("k", 1), _wq(2)), _needs(2)),
    ]
    fences[1] = [(None, (("v", 1), ("wo", 0)), ()), (None, _needs(2), _needs(3))]
    for t in range(HKV + 1):
        pending = list(fences.get(t, []))
        for step in _slot_steps(orders[t], t):
            if step[0] == "fence":
                if pending:
                    pin, waits, starts = pending.pop(0)
                    if pin is not None:
                        p.append(("pin",) + pin)
                    p += wait(*waits) + start(*starts)
            else:
                p.append(step)
                if step[0] == "o" and step[1] == HKV - 1:
                    p += start(("out", step[2]))
        assert not pending
    p += wait(*[("out", j) for j in range(4)])
    return p, len(sem)


_STEPS, _NSEM = _schedule()


def _kernel(x_hbm, k_hbm, v_hbm, wq_hbm, wo_hbm, o_hbm, buf, out_v, sems):
    vals = {}

    def kv_view(base, g):
        return buf.at[pl.ds(base + (g // 4) * 8, 8), :, pl.ds((g % 4) * DH, DH)]

    def copy(name, s):
        sem = sems.at[s]
        kind = name[0]
        if kind == "x":
            cols = pl.ds(name[1] * 128, 128)
            return pltpu.make_async_copy(x_hbm.at[:, :, cols], buf.at[pl.ds(RX, 8), :, cols], sem)
        if kind == "k":
            return pltpu.make_async_copy(k_hbm.at[:, name[1]], kv_view(RK, name[1]), sem)
        if kind == "v":
            return pltpu.make_async_copy(v_hbm.at[:, name[1]], kv_view(RV, name[1]), sem)
        if kind == "wq":
            g, r0, r1, j0, j1 = name[1:]
            ncol = (j1 - j0) * DH
            return pltpu.make_async_copy(
                wq_hbm.at[pl.ds(r0, r1 - r0), :, pl.ds(g * GW + j0 * DH, ncol)],
                buf.at[pl.ds(RWQ + 8 * g + r0, r1 - r0), :, pl.ds(j0 * DH, ncol)], sem)
        if kind == "wo":
            g = name[1]
            return pltpu.make_async_copy(wo_hbm.at[pl.ds(8 * g, 8)], buf.at[pl.ds(RWO + 8 * g, 8)], sem)
        cols = pl.ds(name[1] * 128, 128)
        return pltpu.make_async_copy(out_v.at[:, cols], o_hbm.at[:, cols], sem)

    def x_piece(c):
        if ("x", c) not in vals:
            vals["x", c] = buf[pl.ds(RX, 8), :, pl.ds(c * 128, 128)].reshape(M, 128)
        return vals["x", c]

    def q_first(c):
        w = buf[pl.ds(RWQ + 2 * c, 2), :, :].reshape(128, GW)
        part = jnp.dot(x_piece(c), w, preferred_element_type=f32)
        vals["qacc", c] = part if c == 0 else vals["qacc", c - 1] + part
        if c == 3:
            q = vals["qacc", c].astype(bf16)
            for j in range(REP):
                vals["q", 0, j] = q[:, j * DH:(j + 1) * DH]

    def q_proj(g, j):
        x = jnp.concatenate([x_piece(c) for c in range(4)], axis=1)
        w = buf[pl.ds(RWQ + 8 * g, 8), :, pl.ds(j * DH, DH)].reshape(D, DH)
        vals["q", g, j] = jnp.dot(x, w, preferred_element_type=f32).astype(bf16)

    def qk_softmax(g, b):
        q = jnp.concatenate([vals["q", g, j][b * SQ:(b + 1) * SQ, :] for j in range(REP)], axis=0)
        k = buf[RK + (g // 4) * 8 + b, :, pl.ds((g % 4) * DH, DH)]
        st = jax.lax.dot_general(k, q, (((1,), (1,)), ((), ())), preferred_element_type=f32)
        m = jnp.max(st, axis=0, keepdims=True)
        e = jnp.exp2((st - m) * C)
        l = jnp.sum(e, axis=0, keepdims=True)
        vals["p", g, b] = (e * pl.reciprocal(l, approx=False, full_range=False)).astype(bf16)

    def pv(g, b):
        v = buf[RV + (g // 4) * 8 + b, :, pl.ds((g % 4) * DH, DH)]
        pt = vals.pop(("p", g, b))
        vals["o", g, b] = jax.lax.dot_general(
            pt, v, (((0,), (0,)), ((), ())), preferred_element_type=f32).astype(bf16)

    def out_proj(g, j):
        rows = []
        for b in range(B):
            o = vals["o", g, b]
            rows.append(jnp.concatenate([o[h * SQ:(h + 1) * SQ, :] for h in range(REP)], axis=1))
        o = jnp.concatenate(rows, axis=0)
        w = buf[pl.ds(RWO + 8 * g, 8), :, pl.ds(j * 128, 128)].reshape(GW, 128)
        acc = jnp.dot(o, w, preferred_element_type=f32)
        if g > 0:
            acc = vals["acc", j] + acc
        if g < HKV - 1:
            vals["acc", j] = acc
        else:
            out_v[:, pl.ds(j * 128, 128)] = acc.astype(bf16)

    for step in _STEPS:
        kind = step[0]
        if kind == "start":
            copy(step[1], step[2]).start()
        elif kind == "wait":
            copy(step[1], step[2]).wait()
        elif kind == "q0":
            q_first(step[1])
        elif kind == "q":
            q_proj(step[1], step[2])
        elif kind == "qk":
            qk_softmax(step[1], step[2])
        elif kind == "pv":
            pv(step[1], step[2])
        elif kind == "o":
            out_proj(step[1], step[2])
        else:
            buf[RPAD, pl.ds(0, 16), pl.ds(0, 128)] = vals[step[1]][step[2]:step[2] + 16, 0:128].astype(bf16)


@jax.jit
def pallas_standalone__gqa_block_cached__near_ridge_kernel(
    x: jax.Array,
    k_cache: jax.Array,
    v_cache: jax.Array,
    wq: jax.Array,
    wo: jax.Array,
):
    hbm = pl.BlockSpec(memory_space=pl.ANY)
    out = pl.pallas_call(
        _kernel,
        in_specs=[hbm] * 5,
        out_specs=hbm,
        out_shape=jax.ShapeDtypeStruct((M, D), bf16),
        scratch_shapes=[
            pltpu.VMEM((NR, 64, 512), bf16),
            pltpu.VMEM((M, D), bf16),
            pltpu.SemaphoreType.DMA((_NSEM,)),
        ],
        compiler_params=pltpu.CompilerParams(
            vmem_limit_bytes=100 * 1024 * 1024,
            disable_semaphore_checks=True,
            flags={"XLA_TPU_RESCHEDULE_DMA_DONES": True},
        ),
    )(x, k_cache, v_cache, wq.reshape(8, 64, HQ * DH), wo.reshape(64, 64, D))
    return out.reshape(B, SQ, D)
```

```python
import jax
import jax.numpy as jnp
import numpy as np
import jax.experimental.pallas as pl
import jax.experimental.pallas.tpu as pltpu

B, SQ, D = 8, 64, 512
HQ, HKV, SK, DH = 32, 8, 64, 128
REP = HQ // HKV
GW = REP * DH
M = B * SQ
C = np.float32(DH ** -0.5 * 1.4426950408889634)
bf16 = jnp.bfloat16
f32 = jnp.float32

RX, RWQ, RWO, RK, RV, RPAD, NR = 0, 8, 72, 136, 152, 168, 169


def _wq(g, r0=0, r1=8, j0=0, j1=4):
    return ("wq", g, r0, r1, j0, j1)


def _needs(t):
    r = []
    if t < HKV:
        r.append(("k", t))
    if t + 1 < HKV:
        r.append(_wq(t + 1))
    if t < HKV:
        r.append(("v", t))
    if t >= 1:
        r.append(("wo", t - 1))
    return r


def _slot_steps(order, t):
    steps = []
    for tok in order.split():
        c, arg = tok[0], tok[1:]
        if c == "k":
            steps += [("qk", t, 2 * int(arg)), ("qk", t, 2 * int(arg) + 1)]
        elif c == "q":
            steps.append(("q", t + 1, int(arg)))
        elif c == "p":
            steps += [("pv", t, int(ch)) for ch in arg]
        elif c == "o":
            steps.append(("o", t - 1, int(arg)))
        else:
            steps.append(("fence",))
    return steps


def _schedule():
    sem = {}

    def start(*names):
        return [("start", n, sem.setdefault(n, len(sem))) for n in names]

    def wait(*names):
        return [("wait", n, sem[n]) for n in names]

    def piece(c):
        return (("x", c), _wq(0, 2 * c, 2 * c + 2))

    tile = [_wq(1, 0, 8, j, j + 1) for j in range(REP)]
    copies = [n for c in range(4) for n in piece(c)] + [("k", 0)] + tile + [("v", 0)]
    copies += [n for t in range(1, HKV + 1) for n in _needs(t)]

    row = 320
    p = start(*copies)
    for c in range(4):
        p += wait(*piece(c)) + [("q0", c), ("pin", ("qacc", c), row)]

    orders = {t: "k0 q0 k1 q1 k2 q2 k3 q3 p0123 o0 o1 p4567 o2 | o3" for t in range(1, HKV - 1)}
    orders[0] = "| k0 q0 | k1 q1 | k2 q2 | k3 q3 p0123 p4567 |"
    orders[1] = "k0 q0 k1 q1 k2 q2 k3 q3 | p0123 o0 o1 p4567 o2 | o3"
    orders[HKV - 1] = "k0 o0 k1 o1 k2 o2 k3 p0123 | o3 p4567"
    orders[HKV] = "o0 o1 o2"
    fences = {t: [(None, _needs(t + 1))] for t in range(2, HKV)}
    fences[0] = [
        (None, (("k", 0), tile[0])),
        ((("q", 1, 0), row), (tile[1],)),
        ((("q", 1, 1), row), (tile[2],)),
        ((("q", 1, 2), row), (tile[3], ("v", 0))),
        (None, (("k", 1), _wq(2))),
    ]
    fences[1] = [(None, (("v", 1), ("wo", 0))), (None, _needs(2))]
    for t in range(HKV + 1):
        pending = list(fences.get(t, []))
        for step in _slot_steps(orders[t], t):
            if step[0] == "fence":
                pin, waits = pending.pop(0)
                if pin is not None:
                    p.append(("pin",) + pin)
                p += wait(*waits)
            else:
                p.append(step)
                if step[0] == "o" and step[1] == HKV - 1:
                    p += start(("out", 0, B, step[2]))
    for r in range(0, B, 2):
        p += [("o_rows", r, r + 2, 3)] + start(("out", r, r + 2, 3))
    p += wait(*[n for n in sem if n[0] == "out"])
    return p, len(sem)


_STEPS, _NSEM = _schedule()


def _kernel(x_hbm, k_hbm, v_hbm, wq_hbm, wo_hbm, o_hbm, buf, out_v, acc, sems):
    vals = {}

    def copy(name, s):
        sem = sems.at[s]
        kind = name[0]
        if kind == "x":
            cols = pl.ds(name[1] * 128, 128)
            return pltpu.make_async_copy(x_hbm.at[:, :, cols], buf.at[pl.ds(RX, B), :, cols], sem)
        if kind in ("k", "v"):
            g = name[1]
            src, base = (k_hbm, RK) if kind == "k" else (v_hbm, RV)
            dst = buf.at[pl.ds(base + (g // 4) * B, B), :, pl.ds((g % 4) * DH, DH)]
            return pltpu.make_async_copy(src.at[:, g], dst, sem)
        if kind == "wq":
            g, r0, r1, j0, j1 = name[1:]
            ncol = (j1 - j0) * DH
            return pltpu.make_async_copy(
                wq_hbm.at[pl.ds(r0, r1 - r0), :, pl.ds(g * GW + j0 * DH, ncol)],
                buf.at[pl.ds(RWQ + 8 * g + r0, r1 - r0), :, pl.ds(j0 * DH, ncol)], sem)
        if kind == "wo":
            g = name[1]
            return pltpu.make_async_copy(wo_hbm.at[pl.ds(8 * g, 8)], buf.at[pl.ds(RWO + 8 * g, 8)], sem)
        b0, b1, j = name[1:]
        rows, cols = pl.ds(b0 * SQ, (b1 - b0) * SQ), pl.ds(j * 128, 128)
        return pltpu.make_async_copy(out_v.at[rows, cols], o_hbm.at[rows, cols], sem)

    def x_piece(c):
        if ("x", c) not in vals:
            vals["x", c] = buf[pl.ds(RX, B), :, pl.ds(c * 128, 128)].reshape(M, 128)
        return vals["x", c]

    def q_first(c):
        w = buf[pl.ds(RWQ + 2 * c, 2), :, :].reshape(128, GW)
        part = jnp.dot(x_piece(c), w, preferred_element_type=f32)
        vals["qacc", c] = part if c == 0 else vals["qacc", c - 1] + part
        if c == 3:
            for j in range(REP):
                vals["q", 0, j] = vals["qacc", c][:, j * DH:(j + 1) * DH]

    def q_proj(g, j):
        x = jnp.concatenate([x_piece(c) for c in range(4)], axis=1)
        w = buf[pl.ds(RWQ + 8 * g, 8), :, pl.ds(j * DH, DH)].reshape(D, DH)
        vals["q", g, j] = jnp.dot(x, w, preferred_element_type=f32)

    def qk_softmax(g, b):
        q = jnp.concatenate([vals["q", g, j][b * SQ:(b + 1) * SQ, :] for j in range(REP)], axis=0)
        k = buf[RK + (g // 4) * B + b, :, pl.ds((g % 4) * DH, DH)]
        st = jax.lax.dot_general(k, q.astype(bf16), (((1,), (1,)), ((), ())), preferred_element_type=f32)
        m = jnp.max(st, axis=0, keepdims=True)
        e = jnp.exp2((st - m) * C)
        l = jnp.sum(e, axis=0, keepdims=True)
        vals["p", g, b] = (e * pl.reciprocal(l, approx=False, full_range=False)).astype(bf16)

    def pv(g, b):
        v = buf[RV + (g // 4) * B + b, :, pl.ds((g % 4) * DH, DH)]
        vals["o", g, b] = jax.lax.dot_general(
            vals.pop(("p", g, b)), v, (((0,), (0,)), ((), ())), preferred_element_type=f32)

    def o_rows(g, b0, b1):
        return jnp.concatenate(
            [jnp.concatenate([vals["o", g, b][h * SQ:(h + 1) * SQ, :] for h in range(REP)], axis=1)
             for b in range(b0, b1)], axis=0).astype(bf16)

    def out_proj(g, j, b0=0, b1=B):
        if (b0, b1) == (0, B):
            if ("ofull", g) not in vals:
                vals["ofull", g] = o_rows(g, 0, B)
            o = vals["ofull", g]
        else:
            o = o_rows(g, b0, b1)
        w = buf[pl.ds(RWO + 8 * g, 8), :, pl.ds(j * 128, 128)].reshape(GW, 128)
        c = jnp.dot(o, w, preferred_element_type=f32)
        rows, cols = pl.ds(b0 * SQ, (b1 - b0) * SQ), pl.ds(j * 128, 128)
        if g > 0:
            c = acc[rows, cols] + c
        if g < HKV - 1:
            acc[rows, cols] = c
        else:
            out_v[rows, cols] = c.astype(bf16)

    for step in _STEPS:
        kind = step[0]
        if kind == "start":
            copy(step[1], step[2]).start()
        elif kind == "wait":
            copy(step[1], step[2]).wait()
        elif kind == "q0":
            q_first(step[1])
        elif kind == "q":
            q_proj(step[1], step[2])
        elif kind == "qk":
            qk_softmax(step[1], step[2])
        elif kind == "pv":
            pv(step[1], step[2])
        elif kind == "o":
            out_proj(step[1], step[2])
        elif kind == "o_rows":
            out_proj(HKV - 1, step[3], step[1], step[2])
        else:
            buf[RPAD, pl.ds(0, 16), pl.ds(0, 128)] = vals[step[1]][step[2]:step[2] + 16, 0:128].astype(bf16)


@jax.jit
def pallas_standalone__gqa_block_cached__near_ridge_kernel(
    x: jax.Array,
    k_cache: jax.Array,
    v_cache: jax.Array,
    wq: jax.Array,
    wo: jax.Array,
):
    hbm = pl.BlockSpec(memory_space=pl.ANY)
    out = pl.pallas_call(
        _kernel,
        in_specs=[hbm] * 5,
        out_specs=hbm,
        out_shape=jax.ShapeDtypeStruct((M, D), bf16),
        scratch_shapes=[
            pltpu.VMEM((NR, 64, 512), bf16),
            pltpu.VMEM((M, D), bf16),
            pltpu.VMEM((M, D), f32),
            pltpu.SemaphoreType.DMA((_NSEM,)),
        ],
        compiler_params=pltpu.CompilerParams(
            vmem_limit_bytes=64 * 1024 * 1024,
            disable_semaphore_checks=True,
            flags={"XLA_TPU_RESCHEDULE_DMA_DONES": True},
        ),
    )(x, k_cache, v_cache, wq.reshape(8, 64, HQ * DH), wo.reshape(64, 64, D))
    return out.reshape(B, SQ, D)
```

```python
import jax
import jax.numpy as jnp
import numpy as np
import jax.experimental.pallas as pl
import jax.experimental.pallas.tpu as pltpu

B, SQ, D = 8, 64, 512
HQ, HKV, SK, DH = 32, 8, 64, 128
REP = HQ // HKV
GW = REP * DH
M = B * SQ
C = np.float32(DH ** -0.5 * 1.4426950408889634)
bf16 = jnp.bfloat16
f32 = jnp.float32

RX, RWQ, RWO, RK, RV, RPAD, NR = 0, 8, 72, 136, 152, 168, 169


def _wq(g, r0=0, r1=8, j0=0, j1=4):
    return ("wq", g, r0, r1, j0, j1)


def _needs(t):
    r = []
    if t < HKV:
        r.append(("k", t, 0, B))
    if t + 1 < HKV:
        r.append(_wq(t + 1))
    if t < HKV:
        r.append(("v", t, 0, B))
    if t >= 1:
        r.append(("wo", t - 1))
    return r


def _slot_steps(order, t):
    steps = []
    for tok in order.split():
        c, arg = tok[0], tok[1:]
        if c == "k":
            steps += [("qk", t, 2 * int(arg)), ("qk", t, 2 * int(arg) + 1)]
        elif c == "q":
            steps.append(("q", t + 1, int(arg)))
        elif c == "p":
            steps += [("pv", t, int(ch)) for ch in arg]
        elif c == "o":
            steps.append(("o", t - 1, int(arg)))
        else:
            steps.append(("fence",))
    return steps


def _schedule():
    sem = {}

    def start(*names):
        return [("start", n, sem.setdefault(n, len(sem))) for n in names]

    def wait(*names):
        return [("wait", n, sem[n]) for n in names]

    tile = [_wq(1, 0, 8, j, j + 1) for j in range(REP)]
    kpair = [("k", 0, 2 * i, 2 * i + 2) for i in range(4)]
    copies = [n for c in range(4) for n in (_wq(0, 2 * c, 2 * c + 2), ("x", c, 0), ("x", c, 1))]
    copies += [n for i in range(4) for n in (kpair[i], tile[i])] + [("v", 0, 0, B)]
    copies += [n for t in range(1, HKV + 1) for n in _needs(t)]

    p = start(*copies)
    for c in range(4):
        for h in range(2):
            waits = (_wq(0, 2 * c, 2 * c + 2), ("x", c, 0)) if h == 0 else (("x", c, 1),)
            p += wait(*waits) + [("q0", c, h), ("pin", ("qacc", c, h), 64)]

    orders = {t: "k0 q0 k1 q1 k2 q2 k3 q3 p0123 o0 o1 p4567 o2 | o3" for t in range(1, HKV - 1)}
    orders[0] = "| k0 q0 | k1 q1 | k2 q2 | k3 q3 p0123 p4567 |"
    orders[1] = "k0 q0 k1 q1 k2 q2 k3 q3 | p0123 o0 o1 p4567 o2 | o3"
    orders[HKV - 1] = "k0 o0 k1 o1 k2 o2 k3 p0123 | o3 p4567"
    orders[HKV] = "o0 o1 o2"
    fences = {t: [(None, _needs(t + 1))] for t in range(2, HKV)}
    fences[0] = [
        (None, (kpair[0], tile[0])),
        ((("q", 1, 0), 320), (kpair[1], tile[1])),
        ((("q", 1, 1), 320), (kpair[2], tile[2])),
        ((("q", 1, 2), 320), (kpair[3], tile[3], ("v", 0, 0, B))),
        ((("o", 0, 4), 32), _needs(1)[:2]),
    ]
    fences[1] = [(None, _needs(1)[2:]), (None, _needs(2))]
    for t in range(HKV + 1):
        pending = list(fences.get(t, []))
        for step in _slot_steps(orders[t], t):
            if step[0] == "fence":
                pin, waits = pending.pop(0)
                if pin is not None:
                    p.append(("pin",) + pin)
                p += wait(*waits)
            else:
                p.append(step)
                if step[0] == "o" and step[1] == HKV - 1:
                    p += start(("out", 0, B, step[2]))
    for b0, b1 in ((0, 2), (2, 4), (4, 6), (6, 7), (7, 8)):
        p += [("o_rows", b0, b1, 3)] + start(("out", b0, b1, 3))
    p += wait(*[n for n in sem if n[0] == "out"])
    return p, len(sem)


_STEPS, _NSEM = _schedule()


def _kernel(x_hbm, k_hbm, v_hbm, wq_hbm, wo_hbm, o_hbm, buf, out_v, acc, sems):
    vals = {}

    def copy(name, s):
        sem = sems.at[s]
        kind = name[0]
        if kind == "x":
            c, h = name[1:]
            cols = pl.ds(c * 128, 128)
            return pltpu.make_async_copy(
                x_hbm.at[pl.ds(4 * h, 4), :, cols], buf.at[pl.ds(RX + 4 * h, 4), :, cols], sem)
        if kind in ("k", "v"):
            g, b0, b1 = name[1:]
            src, base = (k_hbm, RK) if kind == "k" else (v_hbm, RV)
            dst = buf.at[pl.ds(base + (g // 4) * B + b0, b1 - b0), :, pl.ds((g % 4) * DH, DH)]
            return pltpu.make_async_copy(src.at[pl.ds(b0, b1 - b0), g], dst, sem)
        if kind == "wq":
            g, r0, r1, j0, j1 = name[1:]
            ncol = (j1 - j0) * DH
            return pltpu.make_async_copy(
                wq_hbm.at[pl.ds(r0, r1 - r0), :, pl.ds(g * GW + j0 * DH, ncol)],
                buf.at[pl.ds(RWQ + 8 * g + r0, r1 - r0), :, pl.ds(j0 * DH, ncol)], sem)
        if kind == "wo":
            g = name[1]
            return pltpu.make_async_copy(wo_hbm.at[pl.ds(8 * g, 8)], buf.at[pl.ds(RWO + 8 * g, 8)], sem)
        b0, b1, j = name[1:]
        rows, cols = pl.ds(b0 * SQ, (b1 - b0) * SQ), pl.ds(j * 128, 128)
        return pltpu.make_async_copy(out_v.at[rows, cols], o_hbm.at[rows, cols], sem)

    def x_piece(c, h):
        if ("x", c, h) not in vals:
            vals["x", c, h] = buf[pl.ds(RX + 4 * h, 4), :, pl.ds(c * 128, 128)].reshape(M // 2, 128)
        return vals["x", c, h]

    def q_first(c, h):
        w = buf[pl.ds(RWQ + 2 * c, 2), :, :].reshape(128, GW)
        part = jnp.dot(x_piece(c, h), w, preferred_element_type=f32)
        vals["qacc", c, h] = part if c == 0 else vals["qacc", c - 1, h] + part
        if c == 3 and h == 1:
            for j in range(REP):
                vals["q", 0, j] = jnp.concatenate(
                    [vals["qacc", 3, hh][:, j * DH:(j + 1) * DH] for hh in range(2)], axis=0)

    def q_proj(g, j):
        x = jnp.concatenate(
            [jnp.concatenate([x_piece(c, h) for c in range(4)], axis=1) for h in range(2)], axis=0)
        w = buf[pl.ds(RWQ + 8 * g, 8), :, pl.ds(j * DH, DH)].reshape(D, DH)
        vals["q", g, j] = jnp.dot(x, w, preferred_element_type=f32)

    def qk_softmax(g, b):
        q = jnp.concatenate([vals["q", g, j][b * SQ:(b + 1) * SQ, :] for j in range(REP)], axis=0)
        k = buf[RK + (g // 4) * B + b, :, pl.ds((g % 4) * DH, DH)]
        st = jax.lax.dot_general(k, q.astype(bf16), (((1,), (1,)), ((), ())), preferred_element_type=f32)
        m = jnp.max(st, axis=0, keepdims=True)
        e = jnp.exp2((st - m) * C)
        l = jnp.sum(e, axis=0, keepdims=True)
        vals["p", g, b] = (e * pl.reciprocal(l, approx=False, full_range=False)).astype(bf16)

    def pv(g, b):
        v = buf[RV + (g // 4) * B + b, :, pl.ds((g % 4) * DH, DH)]
        vals["o", g, b] = jax.lax.dot_general(
            vals.pop(("p", g, b)), v, (((0,), (0,)), ((), ())), preferred_element_type=f32)

    def o_rows(g, b0, b1):
        return jnp.concatenate(
            [jnp.concatenate([vals["o", g, b][h * SQ:(h + 1) * SQ, :] for h in range(REP)], axis=1)
             for b in range(b0, b1)], axis=0).astype(bf16)

    def out_proj(g, j, b0=0, b1=B):
        if (b0, b1) == (0, B):
            if ("ofull", g) not in vals:
                vals["ofull", g] = o_rows(g, 0, B)
            o = vals["ofull", g]
        else:
            o = o_rows(g, b0, b1)
        w = buf[pl.ds(RWO + 8 * g, 8), :, pl.ds(j * 128, 128)].reshape(GW, 128)
        c = jnp.dot(o, w, preferred_element_type=f32)
        rows, cols = pl.ds(b0 * SQ, (b1 - b0) * SQ), pl.ds(j * 128, 128)
        if g > 0:
            c = acc[rows, cols] + c
        if g < HKV - 1:
            acc[rows, cols] = c
        else:
            out_v[rows, cols] = c.astype(bf16)

    for step in _STEPS:
        kind = step[0]
        if kind == "start":
            copy(step[1], step[2]).start()
        elif kind == "wait":
            copy(step[1], step[2]).wait()
        elif kind == "q0":
            q_first(step[1], step[2])
        elif kind == "q":
            q_proj(step[1], step[2])
        elif kind == "qk":
            qk_softmax(step[1], step[2])
        elif kind == "pv":
            pv(step[1], step[2])
        elif kind == "o":
            out_proj(step[1], step[2])
        elif kind == "o_rows":
            out_proj(HKV - 1, step[3], step[1], step[2])
        else:
            buf[RPAD, pl.ds(0, 16), pl.ds(0, 128)] = vals[step[1]][step[2]:step[2] + 16, 0:128].astype(bf16)


@jax.jit
def pallas_standalone__gqa_block_cached__near_ridge_kernel(
    x: jax.Array,
    k_cache: jax.Array,
    v_cache: jax.Array,
    wq: jax.Array,
    wo: jax.Array,
):
    hbm = pl.BlockSpec(memory_space=pl.ANY)
    out = pl.pallas_call(
        _kernel,
        in_specs=[hbm] * 5,
        out_specs=hbm,
        out_shape=jax.ShapeDtypeStruct((M, D), bf16),
        scratch_shapes=[
            pltpu.VMEM((NR, 64, 512), bf16),
            pltpu.VMEM((M, D), bf16),
            pltpu.VMEM((M, D), f32),
            pltpu.SemaphoreType.DMA((_NSEM,)),
        ],
        compiler_params=pltpu.CompilerParams(
            vmem_limit_bytes=64 * 1024 * 1024,
            disable_semaphore_checks=True,
            flags={"XLA_TPU_RESCHEDULE_DMA_DONES": True},
        ),
    )(x, k_cache, v_cache, wq.reshape(8, 64, HQ * DH), wo.reshape(64, 64, D))
    return out.reshape(B, SQ, D)
```
